```python
import jax
import jax.numpy as jnp

def _softmax(x, axis=-1):
    return jax.nn.softmax(x, axis=axis)
def _gelu(x):
    return jax.nn.gelu(x, approximate=True)
def _silu(x):
    return jax.nn.silu(x)
def _sigmoid(x):
    return jax.nn.sigmoid(x)
def _layernorm(x, axis=-1, eps=1e-5):
    m = jnp.mean(x, axis=axis, keepdims=True)
    v = jnp.var(x, axis=axis, keepdims=True)
    return (x - m) / jnp.sqrt(v + eps)
def _scatter_add(tgt, idx, src, axis=0):
    return tgt.at[idx].add(src)
def _segment_sum(src, seg, n):
    return jax.ops.segment_sum(src, seg, n)
class _Rng:
    def __init__(self, key):
        self._k = key
    def _next(self):
        self._k, sub = jax.random.split(self._k)
        return sub
    def normal(self, shape):
        return jax.random.normal(self._next(), shape, dtype=jnp.bfloat16)
    def randint(self, lo, hi, shape):
        return jax.random.randint(self._next(), shape, lo, hi, dtype=jnp.int32)
    def uniform(self, shape, lo=0.0, hi=1.0):
        return jax.random.uniform(self._next(), shape, jnp.bfloat16, lo, hi)
    def permutation(self, n):
        return jax.random.permutation(self._next(), n)


kernel_name = 'gated_mix__sliding_local_dilated__compressed_kv_cla__prompt'

def setup_inputs():
    _rng = _Rng(jax.random.key(int.from_bytes(__import__("os").urandom(4), "little")))
    _w = (lambda a: (lambda t: t.astype(jnp.bfloat16) if jnp.issubdtype(t.dtype, jnp.floating) else t)(jnp.asarray(a)))
    def _A_setup():
        B, S, D = 1, 2048, 576
        return {
            "x": _w((lambda *s: _rng.normal(s) * 0.05)(B, S, D)),
            "wqkv": _w((lambda *s: _rng.normal(s) * 0.05)(D, 3 * D)),
            "wo": _w((lambda *s: _rng.normal(s) * 0.05)(D, D)),
        }
    _A_in = _A_setup()

    def _B_setup():
        B, H, Sq, Sk, D, M = 1, 32, 2048, 2048, 128, 576
        Dc = 4 * D
        return {
            "x": _w((lambda *s: _rng.normal(s) * 0.05)(B, Sq, M)),
            "c_kv": _w((lambda *s: _rng.normal(s) * 0.05)(B, Sk, Dc)),
            "w_q": _w((lambda *s: _rng.normal(s) * 0.05)(M, H, D) * (M ** -0.5)),
            "w_uk": _w((lambda *s: _rng.normal(s) * 0.05)(Dc, H, D) * (Dc ** -0.5)),
            "w_uv": _w((lambda *s: _rng.normal(s) * 0.05)(Dc, H, D) * (Dc ** -0.5)),
            "w_o": _w((lambda *s: _rng.normal(s) * 0.05)(H, D, M) * ((H * D) ** -0.5)),
        }
    _B_in = _B_setup()

    return {
        "A_x": _A_in["x"],
        "A_wqkv": _A_in["wqkv"],
        "A_wo": _A_in["wo"],
        "B_x": _B_in["x"],
        "B_c_kv": _B_in["c_kv"],
        "B_w_q": _B_in["w_q"],
        "B_w_uk": _B_in["w_uk"],
        "B_w_uv": _B_in["w_uv"],
        "B_w_o": _B_in["w_o"],
        "gate_w": _w((lambda *s: _rng.normal(s) * 0.05)(576)),
    }

def reference(A_x, A_wqkv, A_wo, B_x, B_c_kv, B_w_q, B_w_uk, B_w_uv, B_w_o, gate_w):
    def _A_ref(x, wqkv, wo):
        B, S, D = x.shape
        H = 32; Dh = D // H
        W, dil = 8, 2
        qkv = (lambda x, *d: x.transpose(*d))((x @ wqkv).reshape(B, S, 3, H, Dh), 2, 0, 3, 1, 4)
        q, k, v = qkv[0], qkv[1], qkv[2]
        scale = Dh ** -0.5
        pos = jnp.arange(S)
        off = jnp.arange(W) * dil
        idx = pos[:, None] - off[None, :]
        mask = idx >= 0
        idx_c = jnp.where(mask, idx, 0).reshape(-1)
        kg = k[:, :, idx_c, :].reshape(B, H, S, W, Dh)
        vg = v[:, :, idx_c, :].reshape(B, H, S, W, Dh)
        logits = jnp.einsum("bhsd,bhswd->bhsw", q, kg) * scale
        logits = jnp.where(mask[None, None, :, :], logits, -1e9)
        attn = _softmax(logits, axis=-1)
        o = jnp.einsum("bhsw,bhswd->bhsd", attn, vg)
        return (lambda x, *d: x.transpose(*d))(o, 0, 2, 1, 3).reshape(B, S, D) @ wo

    def _B_ref(x, c_kv, w_q, w_uk, w_uv, w_o):
        B, Sq, M = x.shape[0], x.shape[1], x.shape[2]
        Sk = c_kv.shape[1]
        H, D = w_q.shape[1], w_q.shape[2]
        q = jnp.einsum("bqm,mhd->bhqd", x, w_q)
        k = jnp.einsum("bkc,chd->bhkd", c_kv, w_uk)
        v = jnp.einsum("bkc,chd->bhkd", c_kv, w_uv)
        scores = jnp.einsum("bhqd,bhkd->bhqk", q, k) * (D ** -0.5)
        off = Sk - Sq
        qi = jnp.arange(Sq)[:, None]
        kj = jnp.arange(Sk)[None, :]
        cmask = kj <= (qi + off)
        scores = jnp.where(cmask[None, None], scores, -1e9)
        p = _softmax(scores, axis=-1)
        ctx = jnp.einsum("bhqk,bhkd->bhqd", p, v)
        return jnp.einsum("bhqd,hdm->bqm", ctx, w_o)

    x = A_x
    g = _sigmoid((x * gate_w).sum(-1, keepdims=True))
    a = _A_ref(x, A_wqkv, A_wo)
    b = _B_ref(x, B_c_kv, B_w_q, B_w_uk, B_w_uv, B_w_o)
    return g * a + (1 - g) * b
```

```python
import math
import jax
import jax.numpy as jnp
from jax import lax
import jax.experimental.pallas as pl
import jax.experimental.pallas.tpu as pltpu

S, M, C, H, D = 2048, 576, 512, 32, 128
HA, DA, WIN, DIL = 32, 18, 8, 2
MP = 640
BQ = 512
RA = S // H
LOG2E = math.log2(math.e)
NT = (((1,), (1,)), ((), ()))
f32, bf16 = jnp.float32, jnp.bfloat16


def _kernel(xt_ref, wqkv_ref, wo_ref, c_ref, wq_hbm, wk_hbm, wv_hbm, wot_ref, gate_ref, out_ref,
            acc_ref, x_ref, q_ref, k_ref, v_ref, wt_ref, wp_ref, qkv_ref, oa_ref, wq_ref, wk_ref, wv_ref, sems):
    h = pl.program_id(0)

    @pl.when(h == 0)
    def _():
        cps = [pltpu.make_async_copy(src.bitcast(jnp.uint32), dst, sems.at[i])
               for i, (src, dst) in enumerate(((wq_hbm, wq_ref), (wk_hbm, wk_ref), (wv_hbm, wv_ref)))]
        for cp in cps:
            cp.start()
        for c in range(5):
            cw = min(128, M - 128 * c)
            wt_ref[:, pl.ds(0, cw)] = wqkv_ref[pl.ds(128 * c, cw), :].astype(f32).T

            def perm(i, _):
                t, d = i // DA, i % DA
                blk = wt_ref[pl.ds(t * M + d, HA, stride=DA), :]
                wp_ref[pl.ds(pl.multiple_of(t * MP + d * HA, HA), HA), pl.ds(128 * c, cw)] = blk[:, :cw].astype(bf16)
                return 0
            lax.fori_loop(0, 3 * DA, perm, 0, unroll=6)
        for t in range(3):
            wp_ref[pl.ds(t * MP + M, MP - M), :] = jnp.zeros((MP - M, M), bf16)
        qkv_ref[:, pl.ds(0, 16), :] = jnp.zeros((15, 16, 128), f32)

        def proj(i, _):
            r0 = pl.multiple_of(i * 256, 256)
            x = xt_ref[:, pl.ds(r0, 256)].astype(f32).T.astype(bf16)
            x_ref[pl.ds(r0, 256), :] = x
            r = lax.dot_general(x, wp_ref[...], NT, preferred_element_type=f32)
            for c in range(15):
                qkv_ref[c, pl.ds(r0 + 16, 256), :] = r[:, 128 * c:128 * (c + 1)]
            acc_ref[:, pl.ds(r0, 256)] = jnp.zeros((M, 256), f32)
            return 0
        lax.fori_loop(0, S // 256, proj, 0)
        for cp in cps:
            cp.wait()

    a0 = pl.multiple_of(h * RA, RA)
    pos = a0 + lax.broadcasted_iota(jnp.int32, (RA, 128), 0)
    qa = [qkv_ref[c, pl.ds(a0 + 16, RA), :] for c in range(5)]
    ls = []
    for w in range(WIN):
        s = None
        for c in range(5):
            t = qa[c] * qkv_ref[5 + c, pl.ds(a0 + 16 - DIL * w, RA), :]
            s = t if s is None else s + t
        s = s + pltpu.roll(s, 64, 1)
        s = s + pltpu.roll(s, 32, 1)
        s = s * (DA ** -0.5 * LOG2E)
        if w:
            s = jnp.where(pos >= DIL * w, s, -1e9)
        ls.append(s)
    m = ls[0]
    for s in ls[1:]:
        m = jnp.maximum(m, s)
    es = [jnp.exp2(s - m) for s in ls]
    den = es[0]
    for e in es[1:]:
        den = den + e
    inv = 1.0 / den
    for c in range(5):
        o = None
        for w in range(WIN):
            t = es[w] * qkv_ref[10 + c, pl.ds(a0 + 16 - DIL * w, RA), :]
            o = t if o is None else o + t
        oa_ref[pl.ds(a0, RA), pl.ds(128 * c, 128)] = (o * inv).astype(bf16)

    sh = ((h % 2) * 16).astype(jnp.uint32)

    def wload(ref, n):
        u = ref[pl.ds(h // 2, n, stride=H // 2), :]
        return lax.bitcast_convert_type((u >> sh) << 16, f32).astype(bf16)

    wq, wk, wv = wload(wq_ref, M), wload(wk_ref, C), wload(wv_ref, C)

    def proj(i):
        rs = pl.ds(i * BQ, BQ)
        q_ref[rs, :] = (jnp.dot(x_ref[rs, :], wq, preferred_element_type=f32) * (D ** -0.5 * LOG2E)).astype(bf16)
        c = c_ref[rs, :]
        k_ref[rs, :] = jnp.dot(c, wk, preferred_element_type=f32).astype(bf16)
        v_ref[rs, :] = jnp.dot(c, wv, preferred_element_type=f32).astype(bf16)

    NS = BQ // 128
    NB = S // BQ
    tri = lax.broadcasted_iota(jnp.int32, (128, 128), 0) >= lax.broadcasted_iota(jnp.int32, (128, 128), 1)
    proj(0)
    for i in range(NB):
        if i + 1 < NB:
            proj(i + 1)
        r0 = i * BQ
        q = q_ref[pl.ds(r0, BQ), :]
        pieces = [[] for _ in range(NS)]
        if r0:
            sm = lax.dot_general(q, k_ref[pl.ds(0, r0), :], NT, preferred_element_type=f32)
            for r in range(NS):
                pieces[r].append(sm[128 * r:128 * (r + 1)])
        for j in range(NS):
            sj = lax.dot_general(q[128 * j:], k_ref[pl.ds(r0 + 128 * j, 128), :], NT, preferred_element_type=f32)
            for r in range(j, NS):
                t = sj[128 * (r - j):128 * (r - j + 1)]
                pieces[r].append(jnp.where(tri, t, -1e9) if r == j else t)
        ps, ls = [], []
        for r in range(NS):
            s = jnp.concatenate(pieces[r], axis=1) if len(pieces[r]) > 1 else pieces[r][0]
            p = jnp.exp2(s - jnp.max(s, axis=1, keepdims=True))
            ls.append(jnp.sum(p, axis=1, keepdims=True))
            ps.append(p.astype(bf16))
        n0 = r0 + 128
        o = jnp.dot(jnp.concatenate([p[:, :n0] for p in ps], axis=0), v_ref[pl.ds(0, n0), :], preferred_element_type=f32)
        os_ = [o[128 * r:128 * (r + 1)] for r in range(NS)]
        for j in range(1, NS):
            pj = jnp.concatenate([ps[r][:, r0 + 128 * j:r0 + 128 * (j + 1)] for r in range(j, NS)], axis=0)
            oj = jnp.dot(pj, v_ref[pl.ds(r0 + 128 * j, 128), :], preferred_element_type=f32)
            for r in range(j, NS):
                os_[r] = os_[r] + oj[128 * (r - j):128 * (r - j + 1)]
        ctx = jnp.concatenate([os_[r] * (1.0 / ls[r]) for r in range(NS)], axis=0).astype(bf16)
        acc_ref[:, pl.ds(r0, BQ)] += lax.dot_general(wot_ref[...], ctx, NT, preferred_element_type=f32)

    @pl.when(h == H - 1)
    def _():
        wt_ref[pl.ds(M, MP - M), :] = jnp.zeros((MP - M, 128), f32)
        wots = []
        for c in range(5):
            cw = min(128, M - 128 * c)
            wt_ref[pl.ds(MP, M), pl.ds(0, cw)] = wo_ref[:, pl.ds(128 * c, cw)].astype(f32)
            for d in range(DA):
                wt_ref[pl.ds(d * HA, HA), :] = wt_ref[pl.ds(MP + d, HA, stride=DA), :]
            wots.append(wt_ref[pl.ds(0, MP), :].T[:cw].astype(bf16))
        wp_ref[pl.ds(0, M), :] = jnp.concatenate(wots, axis=0)[:, :M]
        gw = jnp.broadcast_to(gate_ref[...], (16, M))

        def fin(i, _):
            cs = pl.ds(pl.multiple_of(i * 256, 256), 256)
            gl = jnp.dot(gw, xt_ref[:, cs], preferred_element_type=f32)[0:1]
            g = 1.0 / (1.0 + jnp.exp(-gl))
            a = lax.dot_general(wp_ref[pl.ds(0, M), :], oa_ref[cs, pl.ds(0, M)], NT, preferred_element_type=f32)
            out_ref[:, cs] = (g * a + (1.0 - g) * acc_ref[:, cs]).astype(out_ref.dtype)
            return 0
        lax.fori_loop(0, S // 256, fin, 0)


@jax.jit
def pallas_gated_mix__sliding_local_dilated__compressed_kv_cla__prompt_kernel(
        A_x, A_wqkv, A_wo, B_x, B_c_kv, B_w_q, B_w_uk, B_w_uv, B_w_o, gate_w):
    del B_x
    full = lambda shape: pl.BlockSpec(shape, lambda i: (0,) * len(shape), pipeline_mode=pl.Buffered(1))
    hbm = pl.BlockSpec(memory_space=pltpu.HBM)
    out = pl.pallas_call(
        _kernel,
        grid=(H,),
        in_specs=[full((M, S)), full((M, 3 * M)), full((M, M)), full((S, C)), hbm, hbm, hbm,
                  pl.BlockSpec((M, D), lambda i: (i, 0)), full((1, M))],
        out_specs=pl.BlockSpec((M, S), lambda i: (0, 0)),
        out_shape=jax.ShapeDtypeStruct((M, S), A_x.dtype),
        scratch_shapes=[pltpu.VMEM((M, S), f32), pltpu.VMEM((S, M), bf16),
                        pltpu.VMEM((S, D), bf16), pltpu.VMEM((S, D), bf16), pltpu.VMEM((S, D), bf16),
                        pltpu.VMEM((3 * M, 128), f32), pltpu.VMEM((3 * MP, M), bf16),
                        pltpu.VMEM((15, S + 16, 128), f32), pltpu.VMEM((S, MP), bf16),
                        pltpu.VMEM((M * H // 2, D), jnp.uint32), pltpu.VMEM((C * H // 2, D), jnp.uint32),
                        pltpu.VMEM((C * H // 2, D), jnp.uint32), pltpu.SemaphoreType.DMA((3,))],
        compiler_params=pltpu.CompilerParams(dimension_semantics=("arbitrary",), vmem_limit_bytes=110 * 1024 * 1024),
    )(A_x.reshape(S, M).T, A_wqkv, A_wo, B_c_kv.reshape(S, C), B_w_q.reshape(M * H, D),
      B_w_uk.reshape(C * H, D), B_w_uv.reshape(C * H, D),
      B_w_o.transpose(0, 2, 1).reshape(H * M, D), gate_w.reshape(1, M))
    return out.T.reshape(1, S, M)
```

```python
import math
import jax
import jax.numpy as jnp
from jax import lax
import jax.experimental.pallas as pl
import jax.experimental.pallas.tpu as pltpu

S, M, C, H, D = 2048, 576, 512, 32, 128
HA, DA, WIN, DIL = 32, 18, 8, 2
MP = 640
BQ = 512
RA = S // H
CH = 256
LOG2E = math.log2(math.e)
NT = (((1,), (1,)), ((), ()))
f32, bf16 = jnp.float32, jnp.bfloat16


def _kernel(xt_hbm, wqkv_hbm, wo_hbm, c_hbm, wq_hbm, wk_hbm, wv_hbm, wot_ref, gate_ref, out_hbm,
            acc_ref, x_ref, q_ref, k_ref, v_ref, wt_ref, wp_ref, qkv_ref, n_ref, wq_ref, wk_ref, wv_ref,
            xt_ref, wqkv_ref, wo_ref, c_ref, wn_ref, woa_ref, g_ref, sems):
    h = pl.program_id(0)
    NC = S // CH

    @pl.when(h == 0)
    def _():
        def cp(i, src, dst):
            return pltpu.make_async_copy(src, dst, sems.at[i])

        def xcp(i):
            cs = pl.ds(pl.multiple_of(i * CH, CH), CH)
            return cp(8 + i, xt_hbm.at[:, cs], xt_ref.at[:, cs])
        wcp = [cp(0, wqkv_hbm.at[pl.ds(0, 256)], wqkv_ref.at[pl.ds(0, 256)]),
               cp(1, wqkv_hbm.at[pl.ds(256, M - 256)], wqkv_ref.at[pl.ds(256, M - 256)]), cp(2, wo_hbm, wo_ref)]
        late = [cp(3, c_hbm, c_ref), cp(4, wq_hbm.bitcast(jnp.uint32), wq_ref),
                cp(5, wk_hbm.bitcast(jnp.uint32), wk_ref), cp(6, wv_hbm.bitcast(jnp.uint32), wv_ref)]
        wcp[0].start()
        wcp[1].start()
        xcp(0).start()
        wcp[2].start()
        for i in range(1, NC):
            xcp(i).start()
        for c_ in late:
            c_.start()
        for t in range(3):
            wp_ref[pl.ds(t * MP + M, MP - M), :] = jnp.zeros((MP - M, M), bf16)
        qkv_ref[:, pl.ds(0, 16), :] = jnp.zeros((15, 16, 128), f32)
        for c in range(5):
            if c in (0, 2):
                wcp[c // 2].wait()
            cw = min(128, M - 128 * c)
            wt_ref[:, pl.ds(0, cw)] = wqkv_ref[pl.ds(128 * c, cw), :].astype(f32).T

            def perm(i, _):
                t, d = i // DA, i % DA
                blk = wt_ref[pl.ds(t * M + d, HA, stride=DA), :]
                wp_ref[pl.ds(pl.multiple_of(t * MP + d * HA, HA), HA), pl.ds(128 * c, cw)] = blk[:, :cw].astype(bf16)
                return 0
            lax.fori_loop(0, 3 * DA, perm, 0, unroll=6)
        gw = jnp.broadcast_to(gate_ref[...], (16, M))

        def xpose(i):
            cs = pl.ds(pl.multiple_of(i * CH, CH), CH)
            xt = xt_ref[:, cs]
            x_ref[cs, :] = xt.astype(f32).T.astype(bf16)
            gl = jnp.dot(gw, xt, preferred_element_type=f32)[0:8]
            g_ref[:, cs] = 1.0 / (1.0 + jnp.exp(-gl))
        xcp(0).wait()
        xpose(0)
        wcp[2].wait()
        wt_ref[pl.ds(M, MP - M), :] = jnp.zeros((MP - M, 128), f32)
        for c in range(5):
            cw = min(128, M - 128 * c)
            wt_ref[pl.ds(MP, M), pl.ds(0, cw)] = wo_ref[:, pl.ds(128 * c, cw)].astype(f32)
            for d in range(DA):
                wt_ref[pl.ds(d * HA, HA), :] = wt_ref[pl.ds(MP + d, HA, stride=DA), :]
            woa_ref[pl.ds(128 * c, cw), :] = wt_ref[pl.ds(0, MP), :].T[:cw, :M].astype(bf16)

        def proj(i, _):
            r0 = pl.multiple_of(i * CH, CH)

            @pl.when(i + 1 < NC)
            def _():
                xcp(i + 1).wait()
            r = lax.dot_general(x_ref[pl.ds(r0, CH), :], wp_ref[...], NT, preferred_element_type=f32)
            xpose(jnp.minimum(i + 1, NC - 1))
            for c in range(15):
                qkv_ref[c, pl.ds(r0 + 16, CH), :] = r[:, 128 * c:128 * (c + 1)]
            acc_ref[:, pl.ds(r0, CH)] = jnp.zeros((M, CH), f32)
            return 0
        lax.fori_loop(0, NC, proj, 0)
        for c_ in late:
            c_.wait()

    def branch_a():
        a0 = pl.multiple_of(h * RA, RA)
        pos = a0 + lax.broadcasted_iota(jnp.int32, (RA, 128), 0)
        qa = [qkv_ref[c, pl.ds(a0 + 16, RA), :] for c in range(5)]
        ls = []
        for w in range(WIN):
            s = None
            for c in range(5):
                t = qa[c] * qkv_ref[5 + c, pl.ds(a0 + 16 - DIL * w, RA), :]
                s = t if s is None else s + t
            s = s + pltpu.roll(s, 64, 1)
            s = s + pltpu.roll(s, 32, 1)
            s = s * (DA ** -0.5 * LOG2E)
            if w:
                s = jnp.where(pos >= DIL * w, s, -1e9)
            ls.append(s)
        m = ls[0]
        for s in ls[1:]:
            m = jnp.maximum(m, s)
        es = [jnp.exp2(s - m) for s in ls]
        den = es[0]
        for e in es[1:]:
            den = den + e
        inv = 1.0 / den
        for c in range(5):
            o = None
            for w in range(WIN):
                t = es[w] * qkv_ref[10 + c, pl.ds(a0 + 16 - DIL * w, RA), :]
                o = t if o is None else o + t
            q_ref[pl.ds(pl.multiple_of((c + 1) * S + a0, RA), RA), :] = (o * inv).astype(bf16)

    def wload(hh):
        sh = ((hh % 2) * 16).astype(jnp.uint32)
        us = [ref[pl.ds(hh // 2, n, stride=H // 2), :] for ref, n in ((wq_ref, M), (wk_ref, C), (wv_ref, C))]
        for t, u in enumerate(us):
            wn_ref[t, pl.ds(0, u.shape[0]), :] = lax.bitcast_convert_type((u >> sh) << 16, f32).astype(bf16)

    def proj(i, dsts, rd):
        rs = pl.ds(i * BQ, BQ)
        dsts[0][rd, :] = (jnp.dot(x_ref[rs, :], wn_ref[0], preferred_element_type=f32) * (D ** -0.5 * LOG2E)).astype(bf16)
        c = c_ref[rs, :]
        dsts[1][rd, :] = jnp.dot(c, wn_ref[1, pl.ds(0, C), :], preferred_element_type=f32).astype(bf16)
        dsts[2][rd, :] = jnp.dot(c, wn_ref[2, pl.ds(0, C), :], preferred_element_type=f32).astype(bf16)

    nxt = [n_ref.at[t] for t in range(3)]

    @pl.when(h == 0)
    def _():
        wload(h)
        proj(0, nxt, pl.ds(0, BQ))

    for t, ref in enumerate((q_ref, k_ref, v_ref)):
        ref[pl.ds(0, BQ), :] = n_ref[t]
    NS = BQ // 128
    NB = S // BQ
    tri = lax.broadcasted_iota(jnp.int32, (128, 128), 0) >= lax.broadcasted_iota(jnp.int32, (128, 128), 1)
    def oproj(i, ctx):
        acc_ref[:, pl.ds(i * BQ, BQ)] += lax.dot_general(wot_ref[...], ctx, NT, preferred_element_type=f32)

    R = 128
    def qk1(r):
        n = (r + 1) * R
        sc = lax.dot_general(q_ref[pl.ds(r * R, R), :], k_ref[pl.ds(0, n), :], NT, preferred_element_type=f32)
        dg = jnp.where(tri, sc[:, n - R:], -1e9)
        sc = jnp.concatenate([sc[:, :n - R], dg], axis=1) if r else dg
        p = jnp.exp2(sc - jnp.max(sc, axis=1, keepdims=True))
        return p.astype(bf16), jnp.sum(p, axis=1, keepdims=True)

    def pv1(r, p, l):
        o = jnp.dot(p, v_ref[pl.ds(0, (r + 1) * R), :], preferred_element_type=f32)
        return (o * (1.0 / l)).astype(bf16)

    NR = S // R
    st, cx = {}, {}
    for t in range(NR + 1):
        if t == 2:
            branch_a()
        if t < NR:
            st[t] = qk1(t)
        if t == NR - NS:
            wload(jnp.minimum(h + 1, H - 1))
        if t % NS == 0 and t < NR:
            i = t // NS
            if i + 1 < NB:
                proj(i + 1, (q_ref, k_ref, v_ref), pl.ds((i + 1) * BQ, BQ))
        if t == NR - 1:
            proj(0, nxt, pl.ds(0, BQ))
        r = t - 1
        if r >= 0:
            cx[r] = pv1(r, *st[r])
            if r % NS == 0 and r:
                oproj(r // NS - 1, jnp.concatenate([cx[u] for u in range(r - NS, r)], axis=0))
    oproj(NB - 1, jnp.concatenate([cx[u] for u in range(NR - NS, NR)], axis=0))

    @pl.when(h == H - 1)
    def _():
        def ocp(i):
            cs = pl.ds(pl.multiple_of(i * CH, CH), CH)
            return pltpu.make_async_copy(xt_ref.at[:, cs], out_hbm.at[:, cs], sems.at[8 + i])

        def fin(i, _):
            r0 = i * CH
            cs = pl.ds(pl.multiple_of(r0, CH), CH)
            oa = jnp.concatenate([q_ref[pl.ds(pl.multiple_of((c + 1) * S + r0, CH), CH), :] for c in range(5)], axis=1)
            a = lax.dot_general(woa_ref[...], oa[:, :M], NT, preferred_element_type=f32)
            g = g_ref[pl.ds(0, 1), cs]
            xt_ref[:, cs] = (g * a + (1.0 - g) * acc_ref[:, cs]).astype(bf16)
            ocp(i).start()
            return 0
        lax.fori_loop(0, NC, fin, 0)
        for i in range(NC):
            ocp(i).wait()


@jax.jit
def pallas_gated_mix__sliding_local_dilated__compressed_kv_cla__prompt_kernel(
        A_x, A_wqkv, A_wo, B_x, B_c_kv, B_w_q, B_w_uk, B_w_uv, B_w_o, gate_w):
    del B_x
    hbm = pl.BlockSpec(memory_space=pltpu.HBM)
    V = pltpu.VMEM
    out = pl.pallas_call(
        _kernel,
        grid=(H,),
        in_specs=[hbm] * 7 + [pl.BlockSpec((M, D), lambda i: (i, 0)), pl.BlockSpec((1, M), lambda i: (0, 0))],
        out_specs=hbm,
        out_shape=jax.ShapeDtypeStruct((M, S), A_x.dtype),
        scratch_shapes=[V((M, S), f32), V((S, M), bf16), V((6 * S, D), bf16), V((S, D), bf16), V((S, D), bf16),
                        V((3 * M, 128), f32), V((3 * MP, M), bf16), V((15, S + 16, 128), f32), V((3, BQ, D), bf16),
                        V((M * H // 2, D), jnp.uint32), V((C * H // 2, D), jnp.uint32), V((C * H // 2, D), jnp.uint32),
                        V((M, S), bf16), V((M, 3 * M), bf16), V((M, M), bf16), V((S, C), bf16),
                        V((3, M, D), bf16), V((M, M), bf16), V((8, S), f32), pltpu.SemaphoreType.DMA((16,))],
        compiler_params=pltpu.CompilerParams(dimension_semantics=("arbitrary",), vmem_limit_bytes=100 * 1024 * 1024),
    )(A_x.reshape(S, M).T, A_wqkv, A_wo, B_c_kv.reshape(S, C), B_w_q.reshape(M * H, D),
      B_w_uk.reshape(C * H, D), B_w_uv.reshape(C * H, D),
      B_w_o.transpose(0, 2, 1).reshape(H * M, D), gate_w.reshape(1, M))
    return out.T.reshape(1, S, M)
```

```python
import math
import jax
import jax.numpy as jnp
from jax import lax
import jax.experimental.pallas as pl
import jax.experimental.pallas.tpu as pltpu

S, M, C, H, D = 2048, 576, 512, 32, 128
HA, DA, WIN, DIL = 32, 18, 8, 2
MP = 640
BQ = 512
RA = S // H
CH = 256
SCHED = 'S0 J1qkv S1 A0,64 P0 S2 P1 S3 P2 S4 J2qkv P3 S5 P4 S6 O0,4 P5 S7 P6 S8 J3qkv P7 S9 P8 S10 O4,8 P9 S11 P10 S12 W P11 S13 P12 S14 O8,12 P13 S15 J0qkv P14 P15 O12,16'
LOG2E = math.log2(math.e)
NEG = -1e9 * LOG2E
NT = (((1,), (1,)), ((), ()))
f32, bf16, u32 = jnp.float32, jnp.bfloat16, jnp.uint32


class _P:
    def __init__(self, ref):
        self.ref = ref

    def _ix(self, start, n):
        half = start // 2
        return pl.ds(half if isinstance(half, int) else pl.multiple_of(half, 8), n // 2)

    def get(self, start, n):
        return pltpu.bitcast(self.ref[self._ix(start, n), :], bf16)

    def put(self, start, val):
        self.ref[self._ix(start, val.shape[0]), :] = pltpu.bitcast(val, jnp.uint32)


def _kernel(xt_hbm, wqkv_hbm, wo_hbm, c_hbm, wq_hbm, wk_hbm, wv_hbm, wot_ref, gate_ref, out_hbm,
            acc_ref, x_ref, q_ref, k_ref, v_ref, wt_ref, wp_ref, qkv_ref, n_ref, wq_ref, wk_ref, wv_ref,
            xt_ref, wqkv_ref, wo_ref, c_ref, wn_ref, woa_ref, g_ref, sems):
    h = pl.program_id(0)
    NC = S // CH

    @pl.when(h == 0)
    def _():
        def cp(i, src, dst):
            return pltpu.make_async_copy(src, dst, sems.at[i])

        def xcp(i):
            cs = pl.ds(pl.multiple_of(i * CH, CH), CH)
            return cp(8 + i, xt_hbm.at[:, cs], xt_ref.at[:, cs])
        wcp = [cp(0, wqkv_hbm.at[pl.ds(0, 256)], wqkv_ref.at[pl.ds(0, 256)]),
               cp(1, wqkv_hbm.at[pl.ds(256, M - 256)], wqkv_ref.at[pl.ds(256, M - 256)]), cp(2, wo_hbm, wo_ref)]
        late = [cp(3, c_hbm.bitcast(jnp.uint32), c_ref), cp(4, wq_hbm.bitcast(jnp.uint32), wq_ref),
                cp(5, wk_hbm.bitcast(jnp.uint32), wk_ref), cp(6, wv_hbm.bitcast(jnp.uint32), wv_ref)]
        wcp[0].start()
        wcp[1].start()
        xcp(0).start()
        wcp[2].start()
        for i in range(1, NC):
            xcp(i).start()
        for c_ in late:
            c_.start()
        for t in range(3):
            wp_ref[pl.ds(t * MP + M, MP - M), :] = jnp.zeros((MP - M, M), bf16)
        qkv_ref[:, pl.ds(0, 16), :] = jnp.zeros((15, 16, 128), f32)
        for c in range(5):
            if c in (0, 2):
                wcp[c // 2].wait()
            cw = min(128, M - 128 * c)
            wt_ref[:, pl.ds(0, cw)] = wqkv_ref[pl.ds(128 * c, cw), :].astype(f32).T

            def perm(i, _):
                t, d = i // DA, i % DA
                blk = wt_ref[pl.ds(t * M + d, HA, stride=DA), :]
                wp_ref[pl.ds(pl.multiple_of(t * MP + d * HA, HA), HA), pl.ds(128 * c, cw)] = blk[:, :cw].astype(bf16)
                return 0
            lax.fori_loop(0, 3 * DA, perm, 0, unroll=6)
        gw = jnp.broadcast_to(gate_ref[...], (16, M))

        def xpose(i):
            cs = pl.ds(pl.multiple_of(i * CH, CH), CH)
            xt = xt_ref[:, cs]
            _P(x_ref).put(i * CH, xt.astype(f32).T.astype(bf16))
            gl = jnp.dot(gw, xt, preferred_element_type=f32)[0:8]
            g_ref[:, cs] = 1.0 / (1.0 + jnp.exp(-gl))
        xcp(0).wait()
        xpose(0)
        wcp[2].wait()
        wt_ref[pl.ds(M, MP - M), :] = jnp.zeros((MP - M, 128), f32)
        for c in range(5):
            cw = min(128, M - 128 * c)
            wt_ref[pl.ds(MP, M), pl.ds(0, cw)] = wo_ref[:, pl.ds(128 * c, cw)].astype(f32)
            for d in range(DA):
                wt_ref[pl.ds(d * HA, HA), :] = wt_ref[pl.ds(MP + d, HA, stride=DA), :]
            woa_ref[pl.ds(128 * c, cw), :] = wt_ref[pl.ds(0, MP), :].T[:cw, :M].astype(bf16)

        def proj(i, _):
            r0 = pl.multiple_of(i * CH, CH)

            @pl.when(i + 1 < NC)
            def _():
                xcp(i + 1).wait()
            r = lax.dot_general(_P(x_ref).get(r0, CH), wp_ref[...], NT, preferred_element_type=f32)
            xpose(jnp.minimum(i + 1, NC - 1))
            for c in range(15):
                qkv_ref[c, pl.ds(r0 + 16, CH), :] = r[:, 128 * c:128 * (c + 1)]
            acc_ref[:, pl.ds(r0, CH)] = jnp.zeros((M, CH), f32)
            return 0
        lax.fori_loop(0, NC, proj, 0)
        for c_ in late:
            c_.wait()

    def branch_a(off, RA):
        a0 = pl.multiple_of(h * (S // H) + off, RA)
        pos = a0 + lax.broadcasted_iota(jnp.int32, (RA, 128), 0)
        qa = [qkv_ref[c, pl.ds(a0 + 16, RA), :] for c in range(5)]
        ls = []
        for w in range(WIN):
            s = None
            for c in range(5):
                t = qa[c] * qkv_ref[5 + c, pl.ds(a0 + 16 - DIL * w, RA), :]
                s = t if s is None else s + t
            s = s + pltpu.roll(s, 64, 1)
            s = s + pltpu.roll(s, 32, 1)
            s = s * (DA ** -0.5 * LOG2E)
            if w:
                s = jnp.where(pos >= DIL * w, s, NEG)
            ls.append(s)
        m = ls[0]
        for s in ls[1:]:
            m = jnp.maximum(m, s)
        es = [jnp.exp2(s - m) for s in ls]
        den = es[0]
        for e in es[1:]:
            den = den + e
        inv = 1.0 / den
        for c in range(5):
            o = None
            for w in range(WIN):
                t = es[w] * qkv_ref[10 + c, pl.ds(a0 + 16 - DIL * w, RA), :]
                o = t if o is None else o + t
            _P(q_ref).put((c + 1) * S + a0, (o * inv).astype(bf16))

    def wload(hh):
        sh = ((hh % 2) * 16).astype(jnp.uint32)
        us = [ref[pl.ds(hh // 2, n, stride=H // 2), :] for ref, n in ((wq_ref, M), (wk_ref, C), (wv_ref, C))]
        for t, u in enumerate(us):
            _P(wn_ref.at[t]).put(0, lax.bitcast_convert_type((u >> sh) << 16, f32).astype(bf16))

    def proj(i, dsts, rd, which='qkv'):
        if 'q' in which:
            _P(dsts[0]).put(rd, (jnp.dot(_P(x_ref).get(i * BQ, BQ), _P(wn_ref.at[0]).get(0, M), preferred_element_type=f32) * (D ** -0.5 * LOG2E)).astype(bf16))
        c = _P(c_ref).get(i * BQ, BQ)
        if 'k' in which:
            _P(dsts[1]).put(rd, jnp.dot(c, _P(wn_ref.at[1]).get(0, C), preferred_element_type=f32).astype(bf16))
        if 'v' in which:
            _P(dsts[2]).put(rd, jnp.dot(c, _P(wn_ref.at[2]).get(0, C), preferred_element_type=f32).astype(bf16))

    nxt = [n_ref.at[t] for t in range(3)]

    @pl.when(h == 0)
    def _():
        wload(h)
        proj(0, nxt, 0)

    for t, ref in enumerate((q_ref, k_ref, v_ref)):
        ref[pl.ds(0, BQ // 2), :] = n_ref[t]
    NS = BQ // 128
    NB = S // BQ
    tri = lax.broadcasted_iota(jnp.int32, (128, 128), 0) >= lax.broadcasted_iota(jnp.int32, (128, 128), 1)
    R = 128
    def qk1(r):
        n = (r + 1) * R
        sc = lax.dot_general(_P(q_ref).get(r * R, R), _P(k_ref).get(0, n), NT, preferred_element_type=f32)
        dg = jnp.where(tri, sc[:, n - R:], NEG)
        sc = jnp.concatenate([sc[:, :n - R], dg], axis=1) if r else dg
        p = jnp.exp2(sc - jnp.max(sc, axis=1, keepdims=True))
        return p.astype(bf16), jnp.sum(p, axis=1, keepdims=True)

    def pv1(r, p, l):
        o = jnp.dot(p, _P(v_ref).get(0, (r + 1) * R), preferred_element_type=f32)
        return (o * (1.0 / l)).astype(bf16)

    NR = S // R
    st, cx = {}, {}
    cur = (q_ref, k_ref, v_ref)
    for op in SCHED.split():
        kind, arg = op[0], op[1:]
        if kind == 'S':
            st[int(arg)] = qk1(int(arg))
        elif kind == 'P':
            cx[int(arg)] = pv1(int(arg), *st[int(arg)])
        elif kind == 'J':
            i = int(arg[0])
            proj(i, cur if i else nxt, i * BQ, arg[1:])
        elif kind == 'W':
            wload(jnp.minimum(h + 1, H - 1))
        elif kind == 'A':
            branch_a(*map(int, arg.split(',')))
        elif kind == 'O':
            lo, hi = map(int, arg.split(','))
            c2 = jnp.concatenate([cx[u] for u in range(lo, hi)], axis=0)
            acc_ref[:, pl.ds(lo * R, (hi - lo) * R)] += lax.dot_general(wot_ref[...], c2, NT, preferred_element_type=f32)

    @pl.when(h == H - 1)
    def _():
        def ocp(i):
            cs = pl.ds(pl.multiple_of(i * CH, CH), CH)
            return pltpu.make_async_copy(xt_ref.at[:, cs], out_hbm.at[:, cs], sems.at[8 + i])

        def fin(i, _):
            r0 = i * CH
            cs = pl.ds(pl.multiple_of(r0, CH), CH)
            oa = jnp.concatenate([_P(q_ref).get((c + 1) * S + r0, CH) for c in range(5)], axis=1)
            a = lax.dot_general(woa_ref[...], oa[:, :M], NT, preferred_element_type=f32)
            g = g_ref[pl.ds(0, 1), cs]
            xt_ref[:, cs] = (g * a + (1.0 - g) * acc_ref[:, cs]).astype(bf16)
            ocp(i).start()
            return 0
        lax.fori_loop(0, NC, fin, 0)
        for i in range(NC):
            ocp(i).wait()


@jax.jit
def pallas_gated_mix__sliding_local_dilated__compressed_kv_cla__prompt_kernel(
        A_x, A_wqkv, A_wo, B_x, B_c_kv, B_w_q, B_w_uk, B_w_uv, B_w_o, gate_w):
    del B_x
    hbm = pl.BlockSpec(memory_space=pltpu.HBM)
    V = pltpu.VMEM
    out = pl.pallas_call(
        _kernel,
        grid=(H,),
        in_specs=[hbm] * 7 + [pl.BlockSpec((M, D), lambda i: (i, 0)), pl.BlockSpec((1, M), lambda i: (0, 0))],
        out_specs=hbm,
        out_shape=jax.ShapeDtypeStruct((M, S), A_x.dtype),
        scratch_shapes=[V((M, S), f32), V((S // 2, M), u32), V((3 * S, D), u32), V((S // 2, D), u32), V((S // 2, D), u32),
                        V((3 * M, 128), f32), V((3 * MP, M), bf16), V((15, S + 16, 128), f32), V((3, BQ // 2, D), u32),
                        V((M * H // 2, D), jnp.uint32), V((C * H // 2, D), jnp.uint32), V((C * H // 2, D), jnp.uint32),
                        V((M, S), bf16), V((M, 3 * M), bf16), V((M, M), bf16), V((S // 2, C), u32),
                        V((3, M // 2, D), u32), V((M, M), bf16), V((8, S), f32), pltpu.SemaphoreType.DMA((16,))],
        compiler_params=pltpu.CompilerParams(dimension_semantics=("arbitrary",), vmem_limit_bytes=100 * 1024 * 1024),
    )(A_x.reshape(S, M).T, A_wqkv, A_wo, B_c_kv.reshape(S, C), B_w_q.reshape(M * H, D),
      B_w_uk.reshape(C * H, D), B_w_uv.reshape(C * H, D),
      B_w_o.transpose(0, 2, 1).reshape(H * M, D), gate_w.reshape(1, M))
    return out.T.reshape(1, S, M)
```
